```python
import os as _os
_os.environ.setdefault("JAX_PLATFORMS", "cpu")
import jax
import jax.numpy as jnp

def _softmax(x, axis=-1):
    return jax.nn.softmax(x, axis=axis)
def _gelu(x):
    return jax.nn.gelu(x, approximate=True)
def _silu(x):
    return jax.nn.silu(x)
def _sigmoid(x):
    return jax.nn.sigmoid(x)
def _layernorm(x, axis=-1, eps=1e-5):
    m = jnp.mean(x, axis=axis, keepdims=True)
    v = jnp.var(x, axis=axis, keepdims=True)
    return (x - m) / jnp.sqrt(v + eps)
def _scatter_add(tgt, idx, src, axis=0):
    return tgt.at[idx].add(src)
def _segment_sum(src, seg, n):
    return jax.ops.segment_sum(src, seg, n)
class _Rng:
    def __init__(self, key):
        self._k = key
    def _next(self):
        self._k, sub = jax.random.split(self._k)
        return sub
    def normal(self, shape):
        return jax.random.normal(self._next(), shape, dtype=jnp.bfloat16)
    def randint(self, lo, hi, shape):
        return jax.random.randint(self._next(), shape, lo, hi, dtype=jnp.int32)
    def uniform(self, shape, lo=0.0, hi=1.0):
        return jax.random.uniform(self._next(), shape, jnp.bfloat16, lo, hi)
    def permutation(self, n):
        return jax.random.permutation(self._next(), n)


kernel_name = 'recurrent_scan__sliding_block__dense_activation_mish__prompt'

def setup_inputs():
    _rng = _Rng(jax.random.key(int.from_bytes(__import__("os").urandom(4), "little")))
    _w = (lambda a: (lambda t: t.astype(jnp.bfloat16) if jnp.issubdtype(t.dtype, jnp.floating) else t)(jnp.asarray(a)))
    def _A_setup():
        B, S, D = 1, 2048, 576
        return {
            "x": _w((lambda *s: _rng.normal(s) * 0.05)(B, S, D)),
            "wqkv": _w((lambda *s: _rng.normal(s) * 0.1)(D, 3 * D)),
            "wo": _w((lambda *s: _rng.normal(s) * 0.1)(D, D)),
        }
    _A_in = _A_setup()

    def _B_setup():
        B, S, D, F = 1, 2048, 576, 4608
        return {
            "x": _w((lambda *s: _rng.normal(s) * 0.05)(B, S, D)),
            "w1": _w((lambda *s: _rng.normal(s) * 0.05)(D, F) * (D ** -0.5)),
            "b1": _w((lambda *s: _rng.normal(s) * 0.05)(F)),
            "w2": _w((lambda *s: _rng.normal(s) * 0.05)(F, D) * (F ** -0.5)),
        }
    _B_in = _B_setup()

    return {
        "A_x": _A_in["x"],
        "A_wqkv": _A_in["wqkv"],
        "A_wo": _A_in["wo"],
        "B_x": _B_in["x"],
        "B_w1": _B_in["w1"],
        "B_b1": _B_in["b1"],
        "B_w2": _B_in["w2"],
    }

def reference(A_x, A_wqkv, A_wo, B_x, B_w1, B_b1, B_w2):
    def _A_ref(x, wqkv, wo):
        B, S, D = x.shape
        H = 32; Dh = D // H; W = 256
        qkv = (lambda x, *d: x.transpose(*d))((x @ wqkv).reshape(B, S, 3, H, Dh), 2, 0, 3, 1, 4)
        q, k, v = qkv[0], qkv[1], qkv[2]
        scores = jnp.einsum("bhqd,bhkd->bhqk", q, k) * (Dh ** -0.5)
        idx = jnp.arange(S)
        mask = (idx[:, None] - idx[None, :] >= 0) & (idx[:, None] - idx[None, :] < W)
        scores = jnp.where(mask[None, None], scores, -1e9)
        p = _softmax(scores, axis=-1)
        o = jnp.einsum("bhqk,bhkd->bhqd", p, v)
        return (lambda x, *d: x.transpose(*d))(o, 0, 2, 1, 3).reshape(B, S, D) @ wo

    def _B_ref(x, w1, b1, w2):
        h = jnp.einsum("bsd,df->bsf", x, w1) + b1
        sp = jnp.log1p(jnp.exp(-jnp.abs(h))) + jnp.where(h > 0, h, jnp.zeros_like(h))
        act = h * jnp.tanh(sp)
        return jnp.einsum("bsf,fd->bsd", act, w2)

    x = A_x
    xn = _layernorm(x, axis=-1)
    s = _A_ref(xn, A_wqkv, A_wo)
    g = _silu(_B_ref(xn, B_w1, B_b1, B_w2))
    return x + s * g
```

```python
import functools

import jax
import jax.numpy as jnp
from jax import lax
import jax.experimental.pallas as pl
import jax.experimental.pallas.tpu as pltpu

S, D, F = 2048, 576, 4608
H, DH, W = 32, 18, 256
TM = 256
NSTEP = S // TM
NG = 8
FC = 1152
NFC = F // FC
QSCALE = (DH ** -0.5) * 1.4426950408889634
NEG = -1e30
F32, BF16 = jnp.float32, jnp.bfloat16
NT = (((1,), (1,)), ((), ()))
TN = (((0,), (0,)), ((), ()))


def _body(first, step, x_ref, wqkv_h, wo_h, w1_h, b1_ref, w2_h, o_ref,
          wqkv, wo, w1, w2, kh, vth, qs, ot, sems):
    def cp_qkv():
        return pltpu.make_async_copy(wqkv_h, wqkv, sems.at[0])

    def cp_wo():
        return pltpu.make_async_copy(wo_h, wo, sems.at[1])

    def cp_w1(c):
        return pltpu.make_async_copy(w1_h.at[:, pl.ds(c * FC, FC)], w1.at[c], sems.at[2 + c])

    def cp_w2(c):
        return pltpu.make_async_copy(w2_h.at[pl.ds(c * FC, FC), :], w2.at[c], sems.at[2 + NFC + c])

    if first:
        cp_qkv().start()
        for c in range(NFC):
            cp_w1(c).start()
            cp_w2(c).start()
        cp_wo().start()
        kh[:, 0:W, :] = jnp.zeros((NG, W, 128), BF16)
        vth[0:2] = jnp.zeros((2, 2 * NG, 48, 128), BF16)

    x = x_ref[...].astype(F32)
    mu = jnp.mean(x, axis=-1, keepdims=True)
    xc = x - mu
    var = jnp.mean(xc * xc, axis=-1, keepdims=True)
    xn = (xc * lax.rsqrt(var + 1e-5)).astype(BF16)

    if first:
        cp_qkv().wait()
    qkv = jnp.dot(xn, wqkv[...], preferred_element_type=F32)
    row0 = pl.multiple_of(step * TM, TM)
    for g in range(NG):
        a = 64 * g
        qs[g] = (qkv[:, a:a + 128] * QSCALE).astype(BF16)
        kh[g, pl.ds(row0 + W, TM), :] = qkv[:, D + a:D + a + 128].astype(BF16)
    vt = qkv[:, 2 * D:3 * D].T
    r8 = lax.broadcasted_iota(jnp.int32, (8, TM), 0)
    ones8 = jnp.ones((8, TM), F32)
    for g in range(NG):
        b = 72 * g
        v0 = jnp.concatenate([vt[b:b + 40], ones8], axis=0).astype(BF16)
        v1 = jnp.concatenate([jnp.where(r8 < 4, 1.0, vt[b + 32:b + 40]), vt[b + 40:b + 72], ones8],
                             axis=0).astype(BF16)
        for t in range(TM // 128):
            vth[step * (TM // 128) + 2 + t, 2 * g] = v0[:, t * 128:(t + 1) * 128]
            vth[step * (TM // 128) + 2 + t, 2 * g + 1] = v1[:, t * 128:(t + 1) * 128]

    lane = lax.broadcasted_iota(jnp.int32, (64, 128), 1)
    rr = lax.broadcasted_iota(jnp.int32, (64, 128), 0)
    upper = rr > (lane & 63)
    lane40 = lax.broadcasted_iota(jnp.int32, (40, 128), 1)
    row40 = lax.broadcasted_iota(jnp.int32, (40, 128), 0)
    zeros64 = jnp.zeros((64, 128), BF16)

    def attn(g, t):
        off = 72 * g - 64 * g
        res = [[None, None], [None, None]]
        for half in range(2):
            q = qs[g, t * 128 + half * 64:t * 128 + half * 64 + 64, :]
            zq = jnp.zeros_like(q)
            qbd = jnp.concatenate(
                [jnp.where((lane >= off + DH * j) & (lane < off + DH * (j + 1)), q, zq) for j in range(4)],
                axis=0)
            kw = kh[g, pl.ds(row0 + t * 128 + half * 64, 320), :]
            s2 = lax.dot_general(kw, qbd, NT, preferred_element_type=F32)
            for p in range(2):
                s = s2[:, p * 128:(p + 1) * 128]
                nskip = max(0, W - (t * 128 + half * 64)) // 64 if first else 0
                blocks = [s[64 * j:64 * j + 64] for j in range(5)]
                if nskip == 0:
                    mid = [jnp.where(upper, blocks[0], blocks[4])] + blocks[1:4]
                else:
                    mid = [jnp.where(upper, NEG, blocks[4])] + blocks[nskip:4]
                m = functools.reduce(jnp.maximum, mid)
                m = jnp.max(m, axis=0, keepdims=True)
                e = [jnp.exp2(b_ - m) for b_ in mid]
                e0 = e[0].astype(BF16)
                if nskip == 0:
                    pb = [jnp.where(upper, e0, zeros64)] + [b_.astype(BF16) for b_ in e[1:]]
                else:
                    pb = [zeros64] * nskip + [b_.astype(BF16) for b_ in e[1:]]
                pb = pb + [jnp.where(upper, zeros64, e0)]
                pb = pb + [zeros64] if half == 0 else [zeros64] + pb
                pt = jnp.concatenate(pb, axis=0)
                c0 = step * (TM // 128) + t
                vw = jnp.concatenate([vth[c0 + j, 2 * g + p] for j in range(3)], axis=1)
                o = jnp.dot(vw, pt, preferred_element_type=F32)
                res[p][half] = o[0:40] * (1.0 / o[40:41])
        outs = []
        for p in range(2):
            a_, b_ = res[p]
            ar, br = pltpu.roll(a_, 64, 1), pltpu.roll(b_, 64, 1)
            first_head = row40 < (DH + 4 * p)
            outs.append(jnp.where(lane40 < 64, jnp.where(first_head, a_, ar), jnp.where(first_head, br, b_)))
        mixed = jnp.where(row40[0:8] < 4, outs[0][32:40], outs[1][0:8])
        ot[72 * g:72 * g + 72, t * 128:(t + 1) * 128] = jnp.concatenate(
            [outs[0][0:32], mixed, outs[1][8:40]], axis=0)

    acc = None
    units = [(g, t) for g in range(NG) for t in range(TM // 128)]
    per = len(units) // NFC
    for c in range(NFC):
        if first:
            cp_w1(c).wait()
        h = jnp.dot(xn, w1[c], preferred_element_type=F32) + b1_ref[:, c * FC:(c + 1) * FC].astype(F32)
        e = jnp.exp(jnp.minimum(h, 20.0))
        n = e * (e + 2.0)
        act = (h * n * pl.reciprocal(n + 2.0, approx=True)).astype(BF16)
        if first:
            cp_w2(c).wait()
        d = jnp.dot(act, w2[c], preferred_element_type=F32)
        acc = d if acc is None else acc + d
        for (g, t) in units[c * per:(c + 1) * per]:
            attn(g, t)

    if first:
        cp_wo().wait()
    sa = lax.dot_general(ot[...].astype(BF16), wo[...], TN, preferred_element_type=F32)
    gate = acc * (1.0 / (1.0 + jnp.exp(-acc)))
    o_ref[...] = (x_ref[...].astype(F32) + sa * gate).astype(o_ref.dtype)


def _kernel(*refs):
    step = pl.program_id(0)

    @pl.when(step == 0)
    def _():
        _body(True, 0, *refs)

    @pl.when(step > 0)
    def _():
        _body(False, step, *refs)


@jax.jit
def pallas_recurrent_scan__sliding_block__dense_activation_mish__prompt_kernel(
    A_x: jax.Array,
    A_wqkv: jax.Array,
    A_wo: jax.Array,
    B_x: jax.Array,
    B_w1: jax.Array,
    B_b1: jax.Array,
    B_w2: jax.Array,
):
    del B_x
    hbm = pl.BlockSpec(memory_space=pl.ANY)
    out = pl.pallas_call(
        _kernel,
        grid=(NSTEP,),
        in_specs=[
            pl.BlockSpec((None, TM, D), lambda i: (0, i, 0)),
            hbm, hbm, hbm,
            pl.BlockSpec((1, F), lambda i: (0, 0)),
            hbm,
        ],
        out_specs=pl.BlockSpec((None, TM, D), lambda i: (0, i, 0)),
        out_shape=jax.ShapeDtypeStruct((1, S, D), A_x.dtype),
        scratch_shapes=[
            pltpu.VMEM((D, 3 * D), BF16),
            pltpu.VMEM((D, D), BF16),
            pltpu.VMEM((NFC, D, FC), BF16),
            pltpu.VMEM((NFC, FC, D), BF16),
            pltpu.VMEM((NG, W + S, 128), BF16),
            pltpu.VMEM((2 + S // 128, 2 * NG, 48, 128), BF16),
            pltpu.VMEM((NG, TM, 128), BF16),
            pltpu.VMEM((D, TM), F32),
            pltpu.SemaphoreType.DMA((2 + 2 * NFC,)),
        ],
        compiler_params=pltpu.CompilerParams(
            dimension_semantics=("arbitrary",),
            vmem_limit_bytes=100 * 1024 * 1024,
        ),
        name="fused_swa_mish",
    )(A_x, A_wqkv, A_wo, B_w1, B_b1.reshape(1, F), B_w2)
    return out
```

```python
import functools

import jax
import jax.numpy as jnp
from jax import lax
import jax.experimental.pallas as pl
import jax.experimental.pallas.tpu as pltpu

S, D, F = 2048, 576, 4608
H, DH, W = 32, 18, 256
TM = 512
NT_ = TM // 128
NSTEP = S // TM
NG = 8
FC = 512
NFC = F // FC
QSCALE = (DH ** -0.5) * 1.4426950408889634
NEG = -1e30
F32, BF16 = jnp.float32, jnp.bfloat16
U32 = jnp.uint32


def _b16(v):
    return pltpu.bitcast(v, BF16)


def _u32(v):
    return pltpu.bitcast(v, U32)


NT = (((1,), (1,)), ((), ()))


def _kernel(x_ref, xp_ref, wqkv_h, wo_h, w1_h, b1_ref, w2_h, o_ref,
            wqkv, wo, w1, w2, kh, vth, qs, ot, wvt, wot, xns, acc, sems):
    step = pl.program_id(0)
    first = step == 0

    def cp_qkv():
        return pltpu.make_async_copy(wqkv_h.bitcast(U32), wqkv, sems.at[0])

    def cp_wo():
        return pltpu.make_async_copy(wo_h.bitcast(U32), wo, sems.at[1])

    def cp_w1(c):
        return pltpu.make_async_copy(w1_h.bitcast(U32).at[:, pl.ds(pl.multiple_of(c * FC, FC), FC)], w1.at[c], sems.at[2 + c])

    def cp_w2(c):
        return pltpu.make_async_copy(w2_h.bitcast(U32).at[:, pl.ds(pl.multiple_of(c * FC, FC), FC)], w2.at[c],
                                     sems.at[2 + NFC + c])

    def spare(g):
        return jnp.where(g == NG - 1, 0, 127)

    lane_t = lax.broadcasted_iota(jnp.int32, (TM, 128), 1)

    @pl.when(first)
    def _():
        cp_qkv().start()
        cp_qkv().wait()
        for c in range(2):
            cp_w1(c).start()
            cp_w2(c).start()
        lane_w = lax.broadcasted_iota(jnp.int32, (W, 128), 1)
        for g in range(NG):
            kh[g, 0:W // 2, :] = _u32(jnp.where(lane_w == spare(g), NEG, 0.0).astype(BF16))
        vth[0:2] = jnp.zeros((2, 2 * NG, 24, 128), U32)

    row0 = pl.multiple_of(step * (TM // 2), TM // 2)

    def norm():
        x = x_ref[...].astype(F32)
        mu = jnp.mean(x, axis=0, keepdims=True)
        xc = x - mu
        var = jnp.mean(xc * xc, axis=0, keepdims=True)
        xnt_f = xc * lax.rsqrt(var + 1e-5)
        xnt = xnt_f.astype(BF16)
        xn = xnt_f.T.astype(BF16)
        xns[...] = _u32(xn)

        return xn, xnt

    def project(xn, xnt):
        qkv = jnp.dot(xn, _b16(wqkv[:, :2 * D]), preferred_element_type=F32)
        for g in range(NG):
            a = 64 * g
            sp = lane_t == spare(g)
            qs[g] = _u32(jnp.where(sp, 1.0, qkv[:, a:a + 128] * QSCALE).astype(BF16))
            kh[g, pl.ds(row0 + W // 2, TM // 2), :] = _u32(jnp.where(sp, 0.0, qkv[:, D + a:D + a + 128]).astype(BF16))
        vt = jnp.dot(_b16(wvt[...]), xnt, preferred_element_type=F32)
        r8 = lax.broadcasted_iota(jnp.int32, (8, TM), 0)
        ones8 = jnp.ones((8, TM), F32)
        for g in range(NG):
            b = 72 * g
            v0 = jnp.concatenate([vt[b:b + 40], ones8], axis=0).astype(BF16)
            v1 = jnp.concatenate([jnp.where(r8 < 4, 1.0, vt[b + 32:b + 40]), vt[b + 40:b + 72], ones8],
                                 axis=0).astype(BF16)
            for t in range(NT_):
                vth[step * NT_ + 2 + t, 2 * g] = _u32(v0)[:, t * 128:(t + 1) * 128]
                vth[step * NT_ + 2 + t, 2 * g + 1] = _u32(v1)[:, t * 128:(t + 1) * 128]

    def scores(g, t, half):
        lane = lax.broadcasted_iota(jnp.int32, (32, 128), 1)
        q = qs[g, t * 64 + half * 32:t * 64 + half * 32 + 32, :]
        qbd = jnp.concatenate(
            [jnp.where(((lane >= 8 * g + DH * j) & (lane < 8 * g + DH * (j + 1))) | (lane == spare(g)),
                       q, jnp.zeros_like(q)) for j in range(4)], axis=0)
        kw = kh[g, pl.ds(pl.multiple_of(row0 + t * 64 + half * 32, 32), 160), :]
        return lax.dot_general(_b16(kw), _b16(qbd), NT, preferred_element_type=F32)

    def probs(s, half):
        lane = lax.broadcasted_iota(jnp.int32, (64, 128), 1)
        rr = lax.broadcasted_iota(jnp.int32, (64, 128), 0)
        upper = rr > (lane & 63)
        z = jnp.zeros((64, 128), F32)
        mid = jnp.concatenate([jnp.where(upper, s[0:64], s[256:320]), s[64:256]], axis=0)
        e = jnp.exp2(mid - jnp.max(mid, axis=0, keepdims=True))
        pb = [jnp.where(upper, e[0:64], 0.0), e[64:], jnp.where(upper, 0.0, e[0:64])]
        pb = pb + [z] if half == 0 else [z] + pb
        return jnp.concatenate(pb, axis=0).astype(BF16)

    def pv(g, t, p, pt):
        c0 = step * NT_ + t
        vw = jnp.concatenate([vth[c0 + j, 2 * g + p] for j in range(3)], axis=1)
        o = jnp.dot(_b16(vw), pt, preferred_element_type=F32)
        return o[0:40] * pl.reciprocal(o[40:41], approx=True)

    def emit(g, t, res):
        lane40 = lax.broadcasted_iota(jnp.int32, (40, 128), 1)
        row40 = lax.broadcasted_iota(jnp.int32, (40, 128), 0)
        outs = []
        for p in range(2):
            a_, b_ = res[(0, p)], res[(1, p)]
            ar, br = pltpu.roll(a_, 64, 1), pltpu.roll(b_, 64, 1)
            first_head = row40 < (DH + 4 * p)
            outs.append(jnp.where(lane40 < 64, jnp.where(first_head, a_, ar), jnp.where(first_head, br, b_)))
        mixed = jnp.where(row40[0:8] < 4, outs[0][32:40], outs[1][0:8])
        ot[pl.ds(pl.multiple_of(72 * g, 8), 72), t * 128:(t + 1) * 128] = jnp.concatenate(
            [outs[0][0:32], mixed, outs[1][8:40]], axis=0)

    def up(c):
        return jnp.dot(_b16(xns[...]), _b16(w1[c]), preferred_element_type=F32) + b1_ref[c].astype(F32)

    def down(c, h):
        e = jnp.exp(jnp.minimum(h, 20.0))
        n = e * (e + 2.0)
        act = (h * n * pl.reciprocal(n + 2.0, approx=True)).astype(BF16)
        return lax.dot_general(_b16(w2[c]), act, NT, preferred_element_type=F32)

    def finish(h, sa):
        f = acc[...] + down(NG, h)
        gate = f * pl.reciprocal(1.0 + jnp.exp(-f), approx=True)
        o_ref[...] = (xp_ref[...].astype(F32) + sa * gate).astype(o_ref.dtype)

    def attn_out():
        return jnp.dot(_b16(wot[...]), ot[...].astype(BF16), preferred_element_type=F32)

    @pl.when(first)
    def _():
        wvt[...] = _u32(_b16(wqkv[:, 2 * D:]).astype(F32).T.astype(BF16))
        project(*norm())

    @pl.when(step == 1)
    def _():
        cp_w1(NG).wait()
        cp_w2(NG).wait()
        cp_wo().wait()
        wot[...] = _u32(_b16(wo[...]).astype(F32).T.astype(BF16))

    @pl.when((step > 0) & (step < NSTEP))
    def _():
        h = up(NG)
        sa = attn_out()
        xn, xnt = norm()
        finish(h, sa)
        project(xn, xnt)

    @pl.when(step == NSTEP)
    def _():
        h = up(NG)
        finish(h, attn_out())

    def loop(g, carry):
        @pl.when(first)
        def _():
            cp_w1(g).wait()
            cp_w2(g).wait()

            @pl.when(g + 2 < NFC)
            def _():
                cp_w1(g + 2).start()
                cp_w2(g + 2).start()

            @pl.when(g + 2 == NFC)
            def _():
                cp_wo().start()

        def sc(ts):
            ss = {(t, half): scores(g, t, half) for t in ts for half in range(2)}
            return {(t, half, p): probs(v[:, p * 128:(p + 1) * 128], half)
                    for (t, half), v in ss.items() for p in range(2)}

        def out(ts, pts):
            for t in ts:
                emit(g, t, {(half, p): pv(g, t, p, pts[(t, half, p)]) for half in range(2) for p in range(2)})

        pa = sc((0, 1))
        h = up(g)
        pb = sc((2, 3))
        out((0, 1), pa)
        out((2, 3), pb)
        acc[...] += down(g, h)
        return carry

    @pl.when(step < NSTEP)
    def _():
        acc[...] = jnp.zeros((D, TM), F32)
        lax.fori_loop(0, NG, loop, 0)


@jax.jit
def pallas_recurrent_scan__sliding_block__dense_activation_mish__prompt_kernel(
    A_x: jax.Array,
    A_wqkv: jax.Array,
    A_wo: jax.Array,
    B_x: jax.Array,
    B_w1: jax.Array,
    B_b1: jax.Array,
    B_w2: jax.Array,
):
    del B_x
    hbm = pl.BlockSpec(memory_space=pltpu.HBM)
    xt = A_x.T[:, :, 0]
    out = pl.pallas_call(
        _kernel,
        grid=(NSTEP + 1,),
        in_specs=[
            pl.BlockSpec((D, TM), lambda i: (0, jnp.minimum(i, NSTEP - 1))),
            pl.BlockSpec((D, TM), lambda i: (0, jnp.maximum(i - 1, 0))),
            hbm, hbm, hbm,
            pl.BlockSpec((NFC, 1, FC), lambda i: (0, 0, 0)),
            hbm,
        ],
        out_specs=pl.BlockSpec((D, TM), lambda i: (0, jnp.maximum(i - 1, 0))),
        out_shape=jax.ShapeDtypeStruct((D, S), A_x.dtype),
        scratch_shapes=[
            pltpu.VMEM((D // 2, 3 * D), U32),
            pltpu.VMEM((D // 2, D), U32),
            pltpu.VMEM((NFC, D // 2, FC), U32),
            pltpu.VMEM((NFC, D // 2, FC), U32),
            pltpu.VMEM((NG, (W + S) // 2, 128), U32),
            pltpu.VMEM((2 + S // 128, 2 * NG, 24, 128), U32),
            pltpu.VMEM((NG, TM // 2, 128), U32),
            pltpu.VMEM((D, TM), F32),
            pltpu.VMEM((D // 2, D), U32),
            pltpu.VMEM((D // 2, D), U32),
            pltpu.VMEM((TM // 2, D), U32),
            pltpu.VMEM((D, TM), F32),
            pltpu.SemaphoreType.DMA((2 + 2 * NFC,)),
        ],
        compiler_params=pltpu.CompilerParams(
            dimension_semantics=("arbitrary",),
            vmem_limit_bytes=100 * 1024 * 1024,
        ),
        name="fused_swa_mish",
    )(xt, xt, A_wqkv, A_wo, B_w1, B_b1.reshape(NFC, 1, FC), B_w2.T)
    return out.T[None]
```

```python
import functools

import jax
import jax.numpy as jnp
from jax import lax
import jax.experimental.pallas as pl
import jax.experimental.pallas.tpu as pltpu

S, D, F = 2048, 576, 4608
H, DH, W = 32, 18, 256
TM = 512
NT_ = TM // 128
NSTEP = S // TM
NG = 8
FC = 512
NFC = F // FC
UN = 4
QSCALE = (DH ** -0.5) * 1.4426950408889634
NEG = -1e30
F32, BF16 = jnp.float32, jnp.bfloat16
U32 = jnp.uint32


def _b16(v):
    return pltpu.bitcast(v, BF16)


def _u32(v):
    return pltpu.bitcast(v, U32)


NT = (((1,), (1,)), ((), ()))


def _kernel(x_h, wqkv_h, wo_h, w1_h, b1_ref, w2_h, o_ref,
            wqkv, wo, w1, w2, kh, vth, qs, ot, wvt, wot, xns, acc, xs, sems, xsem):
    step = pl.program_id(0)
    first = step == 0

    def cp_qkv():
        return pltpu.make_async_copy(wqkv_h.bitcast(U32), wqkv, sems.at[0])

    def cp_wo():
        return pltpu.make_async_copy(wo_h.bitcast(U32), wo, sems.at[1])

    def cp_w1(c):
        return pltpu.make_async_copy(w1_h.bitcast(U32).at[:, pl.ds(pl.multiple_of(c * FC, FC), FC)], w1.at[c], sems.at[2 + c])

    def cp_w2(c):
        return pltpu.make_async_copy(w2_h.bitcast(U32).at[:, pl.ds(pl.multiple_of(c * FC, FC), FC)], w2.at[c],
                                     sems.at[2 + NFC + c])

    def cp_x(i):
        return pltpu.make_async_copy(x_h.at[:, pl.ds(i * TM, TM)], xs.at[i], xsem.at[i])

    def spare(g):
        return jnp.where(g == NG - 1, 0, 127)

    lane_t = lax.broadcasted_iota(jnp.int32, (TM, 128), 1)

    @pl.when(first)
    def _():
        cp_x(0).start()
        cp_w1(0).start()
        cp_qkv().start()
        cp_w2(0).start()
        cp_wo().start()
        lane_w = lax.broadcasted_iota(jnp.int32, (W, 128), 1)
        for g in range(NG):
            kh[g, 0:W // 2, :] = _u32(jnp.where(lane_w == spare(g), NEG, 0.0).astype(BF16))
        vth[0:2] = jnp.zeros((2, H, 16, 128), U32)

    row0 = pl.multiple_of(step * (TM // 2), TM // 2)

    def norm():
        x = xs[step].astype(F32)
        mu = jnp.mean(x, axis=0, keepdims=True)
        xc = x - mu
        var = jnp.mean(xc * xc, axis=0, keepdims=True)
        xnt_f = xc * lax.rsqrt(var + 1e-5)
        xnt = xnt_f.astype(BF16)
        xn = xnt_f.T.astype(BF16)
        xns[...] = _u32(xn)

        return xn, xnt

    def project(xn, xnt):
        qkv = jnp.dot(xn, _b16(wqkv[:, :2 * D]), preferred_element_type=F32)
        for g in range(NG):
            a = 64 * g
            sp = lane_t == spare(g)
            qs[g] = _u32(jnp.where(sp, 1.0, qkv[:, a:a + 128] * QSCALE).astype(BF16))
            kh[g, pl.ds(row0 + W // 2, TM // 2), :] = _u32(jnp.where(sp, 0.0, qkv[:, D + a:D + a + 128]).astype(BF16))
        vt = jnp.dot(_b16(wvt[...]), xnt, preferred_element_type=F32)
        ones8 = jnp.ones((8, TM), F32)
        for hd in range(H):
            b = (DH * hd) // 8 * 8
            v = _u32(jnp.concatenate([vt[b:b + 24], ones8], axis=0).astype(BF16))
            for t in range(NT_):
                vth[step * NT_ + 2 + t, hd] = v[:, t * 128:(t + 1) * 128]

    def scores(g, t, half):
        lane = lax.broadcasted_iota(jnp.int32, (32, 128), 1)
        q = qs[g, t * 64 + half * 32:t * 64 + half * 32 + 32, :]
        qbd = jnp.concatenate(
            [jnp.where(((lane >= 8 * g + DH * j) & (lane < 8 * g + DH * (j + 1))) | (lane == spare(g)),
                       q, jnp.zeros_like(q)) for j in ((0, 1, 2, 3) if half == 0 else (1, 0, 3, 2))], axis=0)
        kw = kh[g, pl.ds(pl.multiple_of(row0 + t * 64 + half * 32, 32), 160), :]
        return lax.dot_general(_b16(kw), _b16(qbd), NT, preferred_element_type=F32)

    def probs(s, half):
        lane = lax.broadcasted_iota(jnp.int32, (64, 128), 1)
        rr = lax.broadcasted_iota(jnp.int32, (64, 128), 0)
        upper = rr > (lane & 63)
        z = jnp.zeros((64, 128), F32)
        mid = jnp.concatenate([jnp.where(upper, s[0:64], s[256:320]), s[64:256]], axis=0)
        e = jnp.exp2(mid - jnp.max(mid, axis=0, keepdims=True))
        pb = [jnp.where(upper, e[0:64], 0.0), e[64:], jnp.where(upper, 0.0, e[0:64])]
        pb = pb + [z] if half == 0 else [z] + pb
        return jnp.concatenate(pb, axis=0).astype(BF16)

    def pv(g, t, p, pa, pb):
        left = lax.broadcasted_iota(jnp.int32, (192, 128), 1) < 64
        pa, pb = _u32(pa), _u32(pb)
        res = []
        for j, pt in enumerate((jnp.where(left, pa, pb), jnp.where(left, pb, pa))):
            c0 = step * NT_ + t
            vw = jnp.concatenate([vth[c0 + i, 4 * g + 2 * p + j] for i in range(3)], axis=1)
            o = jnp.dot(_b16(vw), _b16(pt), preferred_element_type=F32)
            o = o[0:24] * pl.reciprocal(o[24:25], approx=True)
            res.append(pltpu.roll(o, 64, 1) if j else o)
        return res

    def emit(g, t, o):
        row = lax.broadcasted_iota(jnp.int32, (8, 128), 0)
        parts = [o[0][0:16]]
        for j in range(1, 4):
            parts += [jnp.where(row < 2 * j, o[j - 1][16:24], o[j][0:8]), o[j][8:16]]
        parts.append(o[3][16:24])
        ot[pl.ds(pl.multiple_of(72 * g, 8), 72), t * 128:(t + 1) * 128] = jnp.concatenate(parts, axis=0)

    def up(c):
        return jnp.dot(_b16(xns[...]), _b16(w1[c]), preferred_element_type=F32) + b1_ref[c].astype(F32)

    def down(c, h):
        e = jnp.exp(jnp.minimum(h, 20.0))
        n = e * (e + 2.0)
        act = (h * n * pl.reciprocal(n + 2.0, approx=True)).astype(BF16)
        return lax.dot_general(_b16(w2[c]), act, NT, preferred_element_type=F32)

    def finish(sa):
        f = acc[...]
        gate = f * pl.reciprocal(1.0 + jnp.exp(-f), approx=True)
        o_ref[...] = (xs[step - 1].astype(F32) + sa * gate).astype(o_ref.dtype)

    def attn_out():
        return jnp.dot(_b16(wot[...]), ot[...].astype(BF16), preferred_element_type=F32)

    @pl.when(first)
    def _():
        cp_x(0).wait()
        cp_w1(0).wait()
        xn, xnt = norm()
        h = up(0)
        cp_qkv().wait()
        cp_w2(0).wait()
        cp_wo().wait()
        for c in range(1, UN + 1):
            cp_w1(c).start()
            cp_w2(c).start()
        wvt[...] = _u32(_b16(wqkv[:, 2 * D:]).astype(F32).T.astype(BF16))
        wot[...] = _u32(_b16(wo[...]).astype(F32).T.astype(BF16))
        project(xn, xnt)
        acc[...] = down(0, h)

    @pl.when(step == 1)
    def _():
        for i in range(1, NSTEP):
            cp_x(i).wait()

    @pl.when((step > 0) & (step < NSTEP))
    def _():
        finish(attn_out())
        xn, xnt = norm()
        h = up(0)
        project(xn, xnt)
        acc[...] = down(0, h)

    @pl.when(step == NSTEP)
    def _():
        finish(attn_out())

    def loop(i, carry):
        @pl.when(first)
        def _():
            for k in range(1, UN + 1):
                cp_w1(UN * i + k).wait()
                cp_w2(UN * i + k).wait()

            @pl.when(i + 1 < NG // UN)
            def _():
                for k in range(UN + 1, 2 * UN + 1):
                    cp_w1(UN * i + k).start()
                    cp_w2(UN * i + k).start()

            @pl.when(i + 1 == NG // UN)
            def _():
                for j in range(1, NSTEP):
                    cp_x(j).start()

        for k in range(UN):
            group(UN * i + k)
        return carry

    def group(g):
        def sc(ts):
            ss = {(t, half): scores(g, t, half) for t in ts for half in range(2)}
            return {(t, half, p): probs(v[:, p * 128:(p + 1) * 128], half)
                    for (t, half), v in ss.items() for p in range(2)}

        def out(ts, pts):
            for t in ts:
                emit(g, t, [o for p in range(2) for o in pv(g, t, p, pts[(t, 0, p)], pts[(t, 1, p)])])

        pa = sc((0, 1))
        h = up(g + 1)
        pb = sc((2, 3))
        out((0, 1), pa)
        out((2, 3), pb)
        acc[...] += down(g + 1, h)

    @pl.when(step < NSTEP)
    def _():
        lax.fori_loop(0, NG // UN, loop, 0)


@jax.jit
def pallas_recurrent_scan__sliding_block__dense_activation_mish__prompt_kernel(
    A_x: jax.Array,
    A_wqkv: jax.Array,
    A_wo: jax.Array,
    B_x: jax.Array,
    B_w1: jax.Array,
    B_b1: jax.Array,
    B_w2: jax.Array,
):
    del B_x
    hbm = pl.BlockSpec(memory_space=pltpu.HBM)
    xt = A_x.T[:, :, 0]
    out = pl.pallas_call(
        _kernel,
        grid=(NSTEP + 1,),
        in_specs=[
            hbm, hbm, hbm, hbm,
            pl.BlockSpec((NFC, 1, FC), lambda i: (0, 0, 0)),
            hbm,
        ],
        out_specs=pl.BlockSpec((D, TM), lambda i: (0, jnp.maximum(i - 1, 0))),
        out_shape=jax.ShapeDtypeStruct((D, S), A_x.dtype),
        scratch_shapes=[
            pltpu.VMEM((D // 2, 3 * D), U32),
            pltpu.VMEM((D // 2, D), U32),
            pltpu.VMEM((NFC, D // 2, FC), U32),
            pltpu.VMEM((NFC, D // 2, FC), U32),
            pltpu.VMEM((NG, (W + S) // 2, 128), U32),
            pltpu.VMEM((2 + S // 128, H, 16, 128), U32),
            pltpu.VMEM((NG, TM // 2, 128), U32),
            pltpu.VMEM((D, TM), F32),
            pltpu.VMEM((D // 2, D), U32),
            pltpu.VMEM((D // 2, D), U32),
            pltpu.VMEM((TM // 2, D), U32),
            pltpu.VMEM((D, TM), F32),
            pltpu.VMEM((NSTEP, D, TM), BF16),
            pltpu.SemaphoreType.DMA((2 + 2 * NFC,)),
            pltpu.SemaphoreType.DMA((NSTEP,)),
        ],
        compiler_params=pltpu.CompilerParams(
            dimension_semantics=("arbitrary",),
            vmem_limit_bytes=100 * 1024 * 1024,
        ),
        name="fused_swa_mish",
    )(xt, A_wqkv, A_wo, B_w1, B_b1.reshape(NFC, 1, FC), B_w2.T)
    return out.T[None]
```
